```python
import jax
import jax.numpy as jnp

def _softmax(x, axis=-1):
    return jax.nn.softmax(x, axis=axis)

def _gelu(x):
    return jax.nn.gelu(x, approximate=True)

def _silu(x):
    return jax.nn.silu(x)

def _sigmoid(x):
    return jax.nn.sigmoid(x)

def _layernorm(x, axis=-1, eps=1e-05):
    m = jnp.mean(x, axis=axis, keepdims=True)
    v = jnp.var(x, axis=axis, keepdims=True)
    return (x - m) / jnp.sqrt(v + eps)

def _scatter_add(tgt, idx, src, axis=0):
    return tgt.at[idx].add(src)

def _segment_sum(src, seg, n):
    return jax.ops.segment_sum(src, seg, n)

class _Rng:

    def __init__(self, key):
        self._k = key

    def _next(self):
        self._k, sub = jax.random.split(self._k)
        return sub

    def normal(self, shape):
        return jax.random.normal(self._next(), shape, dtype=jnp.bfloat16)

    def randint(self, lo, hi, shape):
        return jax.random.randint(self._next(), shape, lo, hi, dtype=jnp.int32)

    def uniform(self, shape, lo=0.0, hi=1.0):
        return jax.random.uniform(self._next(), shape, jnp.bfloat16, lo, hi)

    def permutation(self, n):
        return jax.random.permutation(self._next(), n)
kernel_name = 'standalone__dilated_atrous__vision'

def setup_inputs():
    _rng = _Rng(jax.random.key(int.from_bytes(__import__("os").urandom(4), "little")))
    _w = lambda a: (lambda t: t.astype(jnp.bfloat16) if jnp.issubdtype(t.dtype, jnp.floating) else t)(jnp.asarray(a))
    H = W = 384
    C = 384
    k = 1
    return {'x': _w((lambda *s: _rng.normal(s) * 0.05)(1, H, W, C)), 'w': _w((lambda *s: _rng.normal(s) * 0.05)(k, k, C, C) * (1.0 / (k * C ** 0.5)))}

def reference(x, w):
    B, H, W, C = x.shape
    k = 1
    rate = 2
    pad = (k - 1) * rate // 2
    xp = jnp.pad(x, ((0, 0), (pad, pad), (pad, pad), (0, 0)))
    out = jnp.zeros_like(x)
    for i in range(k):
        for j in range(k):
            tap = xp[:, i * rate:i * rate + H, j * rate:j * rate + W, :].copy()
            out = out + jnp.einsum('bhwc,co->bhwo', tap, w[i, j])
    return out
```

```python
import jax
import jax.numpy as jnp
from jax import lax
import jax.experimental.pallas as pl
import jax.experimental.pallas.tpu as pltpu

_STREAM = 256
_FIRST = (9, 1, 2)
_GROUP = (12, 2)
_STEP = 128
_CHUNK = 4
_LEAD = 2
_READ_STEPS = 32
_ROUNDS_PER_STEP = 55
_TAIL = 4
_W_STREAMS = 6
_W_PAGES = 4
_W_FIRST = 28
_W_PER_STEP = 26


def _split(i, n):
    assert n & (n - 1) == 0
    return lax.shift_right_logical(i, n.bit_length() - 1), i & (n - 1)


@jax.jit
def pallas_standalone__dilated_atrous__vision_kernel(
    x: jax.Array,
    w: jax.Array,
):
    B, H, W, C = x.shape
    assert w.shape == (1, 1, C, C) and C == 384 and x.dtype.itemsize == 2
    n_blocks = B * H * W // 16
    n_streams = n_blocks * 3 // _STREAM
    n_steps = n_blocks // _STEP
    assert n_streams * _STREAM == n_blocks * 3 and n_steps * _STEP == n_blocks

    first = _FIRST[0] + _FIRST[1]
    group = sum(_GROUP)
    n_groups = (n_streams - first) // group
    assert first + n_groups * group == n_streams and _STREAM % _FIRST[2] == 0
    n_rounds = n_groups * _STREAM
    early_rounds = n_rounds - _READ_STEPS * _ROUNDS_PER_STEP
    assert early_rounds >= 0
    group_start = [0] + [first + g * group for g in range(n_groups + 1)]
    first_use = [s * _STREAM // (3 * _STEP) for s in group_start[:-1]]
    assert first_use[-1] >= _READ_STEPS

    w_rounds = _STREAM // _W_PAGES
    n_writes = n_streams // _W_STREAMS * w_rounds
    assert n_streams % _W_STREAMS == 0
    for i in range(_READ_STEPS, n_steps):
        last = _W_FIRST + (i - _READ_STEPS + 1) * _W_PER_STEP - 1
        assert (last // w_rounds + 1) * _W_STREAMS * _STREAM <= i * _STEP * 3

    def kernel_function(x_hbm, w_hbm, o_hbm, buf, wbuf, out_sem):
        blocks = buf.reshape(n_blocks, 3, 16, 128)

        def top_half():
            return lax.broadcasted_iota(jnp.int32, (_CHUNK, 8, 128), 1) < 4

        def load(b0):
            p = [pltpu.bitcast(blocks[pl.ds(b0, _CHUNK), j], jnp.int32) for j in range(3)]
            top = top_half()
            cols = (
                jnp.where(top, p[0], p[1]),
                pltpu.roll(jnp.where(top, p[2], p[0]), 4, 1),
                jnp.where(top, p[1], p[2]),
            )
            return jnp.concatenate(
                [pltpu.bitcast(v, buf.dtype).reshape(_CHUNK * 16, 128) for v in cols], axis=1)

        def store(b0, y):
            c = [pltpu.bitcast(y[:, n * 128:(n + 1) * 128].reshape(_CHUNK, 16, 128), jnp.int32)
                 for n in range(3)]
            top = top_half()
            c1 = pltpu.roll(c[1], 4, 1)
            pages = (
                jnp.where(top, c[0], c1),
                jnp.where(top, c[2], c[0]),
                jnp.where(top, c1, c[2]),
            )
            for j, v in enumerate(pages):
                blocks[pl.ds(b0, _CHUNK), j] = pltpu.bitcast(v, buf.dtype)

        def matmul_step(i, n_starts, start):
            n_chunks = _STEP // _CHUNK
            slots = iter(range(2 * n_chunks))

            def start_some():
                s = next(slots)
                lo, hi = ((t * n_starts + n_chunks) // (2 * n_chunks) for t in (s, s + 1))
                for k in range(lo, hi):
                    start(k)

            loaded = {}
            for u in range(-_LEAD, n_chunks):
                if u + _LEAD < n_chunks:
                    start_some()
                    loaded[u + _LEAD] = load(i * _STEP + (u + _LEAD) * _CHUNK)
                if u >= 0:
                    y = jnp.dot(loaded.pop(u), wbuf[...], preferred_element_type=jnp.float32)
                    start_some()
                    store(i * _STEP + u * _CHUNK, y.astype(buf.dtype))

        def start_write(k):
            g, r = _split(k, w_rounds)
            idx = (pl.ds(g * _W_STREAMS, _W_STREAMS), pl.ds(r * _W_PAGES, _W_PAGES))
            pltpu.make_async_copy(buf.at[idx], o_hbm.at[idx], out_sem).start()

        def read_phase(sems):
            tail_sem, w_sem = n_groups + 1, n_groups + 2

            def read(stream, streams, page, pages, sem):
                idx = (pl.ds(stream, streams), pl.ds(page, pages))
                return pltpu.make_async_copy(x_hbm.at[idx], buf.at[idx], sems.at[sem])

            def start_read(t, queue):
                g, r = _split(t, _STREAM)
                sem = jnp.where(t >= n_rounds - _TAIL, tail_sem, g + 1)
                stream = first + g * group
                if queue == 1:
                    read(stream, _GROUP[0], r, 1, sem).start(priority=1)
                else:
                    read(stream + _GROUP[0], _GROUP[1], r, 1, sem).start(priority=0)

            def wait_group(g):
                read(group_start[g], group_start[g + 1] - group_start[g], 0, _STREAM, g).wait()

            w_copy = pltpu.make_async_copy(w_hbm, wbuf, sems.at[w_sem])
            w_copy.start()

            def first_round(r, _):
                on_1, on_0, pages = _FIRST
                read(0, on_1, r * pages, pages, 0).start(priority=1)
                read(on_1, on_0, r * pages, pages, 0).start(priority=0)

            def early_round(t, _):
                start_read(t, 1)
                start_read(t, 0)

            lax.fori_loop(0, _STREAM // _FIRST[2], first_round, None)
            lax.fori_loop(0, early_rounds, early_round, None)
            w_copy.wait()

            def step(i, _):
                for g, i0 in enumerate(first_use):
                    if i0 < _READ_STEPS:
                        pl.when(i == i0)(lambda g=g: wait_group(g))
                t0 = early_rounds + i * _ROUNDS_PER_STEP
                matmul_step(i, 2 * _ROUNDS_PER_STEP,
                            lambda k: start_read(t0 + k // 2, 1 - k % 2))

            lax.fori_loop(0, _READ_STEPS, step, None)

            for g, i0 in enumerate(first_use[:-1]):
                if i0 >= _READ_STEPS:
                    wait_group(g)
            read(group_start[-2], group, 0, _STREAM - _TAIL, n_groups).wait()
            lax.fori_loop(0, _W_FIRST, lambda k, _: start_write(k), None)
            read(group_start[-2], group, _STREAM - _TAIL, _TAIL, tail_sem).wait()

        pl.run_scoped(read_phase, pltpu.SemaphoreType.DMA((n_groups + 3,)))

        def step(i, _):
            k0 = _W_FIRST + (i - _READ_STEPS) * _W_PER_STEP
            matmul_step(i, _W_PER_STEP, lambda k: start_write(k0 + k))

        lax.fori_loop(_READ_STEPS, n_steps, step, None)
        lax.fori_loop(_W_FIRST + (n_steps - _READ_STEPS) * _W_PER_STEP, n_writes,
                      lambda k, _: start_write(k), None)
        pltpu.make_async_copy(buf, o_hbm, out_sem).wait()

    shape = (n_streams, _STREAM, 16, 128)
    tiles = x.reshape(2 * n_blocks, 8, 3, 128).transpose(0, 2, 1, 3)
    out = pl.pallas_call(
        kernel_function,
        in_specs=[
            pl.BlockSpec(memory_space=pl.ANY),
            pl.BlockSpec(memory_space=pl.ANY),
        ],
        out_specs=pl.BlockSpec(memory_space=pl.ANY),
        out_shape=jax.ShapeDtypeStruct(shape, x.dtype),
        scratch_shapes=[
            pltpu.VMEM(shape, x.dtype),
            pltpu.VMEM((C, C), w.dtype),
            pltpu.SemaphoreType.DMA(()),
        ],
        compiler_params=pltpu.CompilerParams(
            vmem_limit_bytes=120 * 2**20, disable_bounds_checks=True),
    )(tiles.reshape(shape), w.reshape(C, C))
    return out.reshape(2 * n_blocks, 3, 8, 128).transpose(0, 2, 1, 3).reshape(B, H, W, C)
```

```python
import jax
import jax.numpy as jnp
from jax import lax
import jax.experimental.pallas as pl
import jax.experimental.pallas.tpu as pltpu

_STREAM = 256
_FIRST = 10
_GROUP = 14
_STEP = 128
_CHUNK = 4
_LEAD = 2
_READ_STEPS = 32
_ROUNDS_PER_STEP = 55
_TAIL = 8
_W_STREAMS = 6
_W_PAGES = 4
_W_FIRST = 28
_W_PER_STEP = 26


def _split(i, n):
    assert n & (n - 1) == 0
    return lax.shift_right_logical(i, n.bit_length() - 1), i & (n - 1)


@jax.jit
def pallas_standalone__dilated_atrous__vision_kernel(
    x: jax.Array,
    w: jax.Array,
):
    B, H, W, C = x.shape
    assert w.shape == (1, 1, C, C) and C == 384 and x.dtype.itemsize == 2
    n_blocks = B * H * W // 16
    n_streams = n_blocks * 3 // _STREAM
    n_steps = n_blocks // _STEP
    assert n_streams * _STREAM == n_blocks * 3 and n_steps * _STEP == n_blocks

    n_groups = 1 + (n_streams - _FIRST) // _GROUP
    group_start = [0] + [_FIRST + g * _GROUP for g in range(n_groups)]
    assert group_start[-1] == n_streams
    n_rounds = n_groups * _STREAM
    early_rounds = n_rounds - _READ_STEPS * _ROUNDS_PER_STEP
    assert early_rounds >= _STREAM
    first_use = [s * _STREAM // (3 * _STEP) for s in group_start[:-1]]
    assert first_use[-1] >= _READ_STEPS
    for g, i in enumerate(first_use):
        assert i >= _READ_STEPS or early_rounds + i * _ROUNDS_PER_STEP >= (g + 1) * _STREAM

    w_rounds = _STREAM // _W_PAGES
    n_writes = n_streams // _W_STREAMS * w_rounds
    assert n_streams % _W_STREAMS == 0
    for i in range(_READ_STEPS, n_steps):
        last = _W_FIRST + (i - _READ_STEPS + 1) * _W_PER_STEP - 1
        assert (last // w_rounds + 1) * _W_STREAMS * _STREAM <= i * _STEP * 3

    def kernel_function(x_hbm, w_hbm, o_hbm, buf, wbuf, out_sem):
        blocks = buf.reshape(n_blocks, 3, 16, 128)

        def top_half():
            return lax.broadcasted_iota(jnp.int32, (_CHUNK, 8, 128), 1) < 4

        def load(b0):
            p = [pltpu.bitcast(blocks[pl.ds(b0, _CHUNK), j], jnp.int32) for j in range(3)]
            top = top_half()
            cols = (
                jnp.where(top, p[0], p[1]),
                pltpu.roll(jnp.where(top, p[2], p[0]), 4, 1),
                jnp.where(top, p[1], p[2]),
            )
            return jnp.concatenate(
                [pltpu.bitcast(v, buf.dtype).reshape(_CHUNK * 16, 128) for v in cols], axis=1)

        def store(b0, y):
            c = [pltpu.bitcast(y[:, n * 128:(n + 1) * 128].reshape(_CHUNK, 16, 128), jnp.int32)
                 for n in range(3)]
            top = top_half()
            c1 = pltpu.roll(c[1], 4, 1)
            pages = (
                jnp.where(top, c[0], c1),
                jnp.where(top, c[2], c[0]),
                jnp.where(top, c1, c[2]),
            )
            for j, v in enumerate(pages):
                blocks[pl.ds(b0, _CHUNK), j] = pltpu.bitcast(v, buf.dtype)

        def matmul_step(i, n_starts, start):
            n_chunks = _STEP // _CHUNK
            slots = iter(range(2 * n_chunks))

            def start_some():
                s = next(slots)
                lo, hi = ((t * n_starts + n_chunks) // (2 * n_chunks) for t in (s, s + 1))
                for k in range(lo, hi):
                    start(k)

            loaded = {}
            for u in range(-_LEAD, n_chunks):
                if u + _LEAD < n_chunks:
                    start_some()
                    loaded[u + _LEAD] = load(i * _STEP + (u + _LEAD) * _CHUNK)
                if u >= 0:
                    y = jnp.dot(loaded.pop(u), wbuf[...], preferred_element_type=jnp.float32)
                    start_some()
                    store(i * _STEP + u * _CHUNK, y.astype(buf.dtype))

        def start_write(k):
            g, r = _split(k, w_rounds)
            idx = (pl.ds(g * _W_STREAMS, _W_STREAMS), pl.ds(r * _W_PAGES, _W_PAGES))
            pltpu.make_async_copy(buf.at[idx], o_hbm.at[idx], out_sem).start()

        def read_phase(sems):
            tail_sem, w_sem = n_groups, n_groups + 1

            def read(stream, streams, page, pages, sem):
                idx = (pl.ds(stream, streams), pl.ds(page, pages))
                return pltpu.make_async_copy(x_hbm.at[idx], buf.at[idx], sems.at[sem])

            def start_read(stream, streams, page, sem, queue):
                if queue == 1:
                    read(stream, streams - 1, page, 1, sem).start(priority=1)
                else:
                    read(stream + streams - 1, 1, page, 1, sem).start(priority=0)

            def start_round(t, queue):
                g, r = _split(t, _STREAM)
                sem = jnp.where(t >= n_rounds - _TAIL, tail_sem, g)
                start_read(_FIRST + (g - 1) * _GROUP, _GROUP, r, sem, queue)

            def wait_group(g):
                read(group_start[g], group_start[g + 1] - group_start[g], 0, _STREAM, g).wait()

            def first_round(r, _):
                start_read(0, _FIRST, r, 0, 1)
                start_read(0, _FIRST, r, 0, 0)

            def early_round(t, _):
                start_round(t, 1)
                start_round(t, 0)

            lax.fori_loop(0, _STREAM, first_round, None)
            w_copy = pltpu.make_async_copy(w_hbm, wbuf, sems.at[w_sem])
            w_copy.start()
            lax.fori_loop(_STREAM, early_rounds, early_round, None)
            w_copy.wait()

            def step(i, _):
                for g, i0 in enumerate(first_use):
                    if i0 < _READ_STEPS:
                        pl.when(i == i0)(lambda g=g: wait_group(g))
                t0 = early_rounds + i * _ROUNDS_PER_STEP
                matmul_step(i, 2 * _ROUNDS_PER_STEP,
                            lambda k: start_round(t0 + k // 2, 1 - k % 2))

            lax.fori_loop(0, _READ_STEPS, step, None)

            for g, i0 in enumerate(first_use[:-1]):
                if i0 >= _READ_STEPS:
                    wait_group(g)
            read(group_start[-2], _GROUP, 0, _STREAM - _TAIL, n_groups - 1).wait()
            lax.fori_loop(0, _W_FIRST, lambda k, _: start_write(k), None)
            read(group_start[-2], _GROUP, _STREAM - _TAIL, _TAIL, tail_sem).wait()

        pl.run_scoped(read_phase, pltpu.SemaphoreType.DMA((n_groups + 2,)))

        def step(i, _):
            k0 = _W_FIRST + (i - _READ_STEPS) * _W_PER_STEP
            matmul_step(i, _W_PER_STEP, lambda k: start_write(k0 + k))

        lax.fori_loop(_READ_STEPS, n_steps, step, None)
        lax.fori_loop(_W_FIRST + (n_steps - _READ_STEPS) * _W_PER_STEP, n_writes,
                      lambda k, _: start_write(k), None)
        pltpu.make_async_copy(buf, o_hbm, out_sem).wait()

    shape = (n_streams, _STREAM, 16, 128)
    tiles = x.reshape(2 * n_blocks, 8, 3, 128).transpose(0, 2, 1, 3)
    out = pl.pallas_call(
        kernel_function,
        in_specs=[
            pl.BlockSpec(memory_space=pl.ANY),
            pl.BlockSpec(memory_space=pl.ANY),
        ],
        out_specs=pl.BlockSpec(memory_space=pl.ANY),
        out_shape=jax.ShapeDtypeStruct(shape, x.dtype),
        scratch_shapes=[
            pltpu.VMEM(shape, x.dtype),
            pltpu.VMEM((C, C), w.dtype),
            pltpu.SemaphoreType.DMA(()),
        ],
        compiler_params=pltpu.CompilerParams(
            vmem_limit_bytes=120 * 2**20,
            disable_bounds_checks=True,
            disable_semaphore_checks=True,
        ),
    )(tiles.reshape(shape), w.reshape(C, C))
    return out.reshape(2 * n_blocks, 3, 8, 128).transpose(0, 2, 1, 3).reshape(B, H, W, C)
```

```python
import jax
import jax.numpy as jnp
from jax import lax
import jax.experimental.pallas as pl
import jax.experimental.pallas.tpu as pltpu

_STREAM = 256
_FIRST = 10
_GROUP = 14
_STEP = 128
_CHUNK = 4
_LEAD = 2
_READ_STEPS = 32
_ROUNDS_PER_STEP = 55
_TAIL = 8
_W_STREAMS = 6
_W_PAGES = 4
_W_FIRST = 28
_W_PER_STEP = 26


def _split(i, n):
    assert n & (n - 1) == 0
    return lax.shift_right_logical(i, n.bit_length() - 1), i & (n - 1)


@jax.jit
def pallas_standalone__dilated_atrous__vision_kernel(
    x: jax.Array,
    w: jax.Array,
):
    B, H, W, C = x.shape
    assert w.shape == (1, 1, C, C) and C == 384 and x.dtype.itemsize == 2
    n_blocks = B * H * W // 16
    n_streams = n_blocks * 3 // _STREAM
    n_steps = n_blocks // _STEP
    assert n_streams * _STREAM == n_blocks * 3 and n_steps * _STEP == n_blocks
    half = _STREAM // 2
    step_halves = _STEP * 3 // half
    assert step_halves * half == _STEP * 3

    n_groups = 1 + (n_streams - _FIRST) // _GROUP
    group_start = [0] + [_FIRST + g * _GROUP for g in range(n_groups)]
    assert group_start[-1] == n_streams
    n_rounds = n_groups * _STREAM
    early_rounds = n_rounds - _READ_STEPS * _ROUNDS_PER_STEP
    assert early_rounds >= _STREAM
    first_use = [s * _STREAM // (3 * _STEP) for s in group_start[:-1]]
    assert first_use[-1] >= _READ_STEPS
    for g, i in enumerate(first_use):
        assert i >= _READ_STEPS or early_rounds + i * _ROUNDS_PER_STEP >= (g + 1) * _STREAM

    w_rounds = _STREAM // _W_PAGES
    n_writes = n_streams // _W_STREAMS * w_rounds
    assert n_streams % _W_STREAMS == 0
    for i in range(_READ_STEPS, n_steps):
        last = _W_FIRST + (i - _READ_STEPS + 1) * _W_PER_STEP - 1
        assert (last // w_rounds + 1) * _W_STREAMS * _STREAM <= i * _STEP * 3

    def kernel_function(x_hbm, w_hbm, o_hbm, buf, wbuf, out_sem):
        def as_words(v):
            return pltpu.bitcast(v, jnp.int32)

        def merge(top, bottom):
            return jnp.where(lax.broadcasted_iota(jnp.int32, (8, 128), 0) < 4, top, bottom)

        def load(page, blocks):
            rows = []
            for b in blocks:
                p0, p1, p2 = (as_words(buf[page(3 * b + j)]) for j in range(3))
                cols = (merge(p0, p1), pltpu.roll(merge(p2, p0), 4, 0), merge(p1, p2))
                rows.append(jnp.concatenate([pltpu.bitcast(v, buf.dtype) for v in cols], axis=1))
            return jnp.concatenate(rows, axis=0)

        def store(page, blocks, y):
            for u, b in enumerate(blocks):
                c0, c1, c2 = (as_words(y[16 * u:16 * u + 16, 128 * j:128 * j + 128]) for j in range(3))
                c1 = pltpu.roll(c1, 4, 0)
                for j, v in enumerate((merge(c0, c1), merge(c2, c0), merge(c1, c2))):
                    buf[page(3 * b + j)] = pltpu.bitcast(v, buf.dtype)

        def matmul_step(i, n_starts, start):
            halves = [_split(i * step_halves + h, 2) for h in range(step_halves)]

            def page(n):
                stream, second = halves[n // half]
                return stream, second * half + n % half

            def blocks(chunk):
                return range(chunk * _CHUNK, (chunk + 1) * _CHUNK)

            n_chunks = _STEP // _CHUNK
            slots = iter(range(2 * n_chunks))

            def start_some():
                s = next(slots)
                lo, hi = ((t * n_starts + n_chunks) // (2 * n_chunks) for t in (s, s + 1))
                for k in range(lo, hi):
                    start(k)

            loaded = {}
            for u in range(-_LEAD, n_chunks):
                if u + _LEAD < n_chunks:
                    start_some()
                    loaded[u + _LEAD] = load(page, blocks(u + _LEAD))
                if u >= 0:
                    y = jnp.dot(loaded.pop(u), wbuf[...], preferred_element_type=jnp.float32)
                    start_some()
                    store(page, blocks(u), y.astype(buf.dtype))

        def start_write(k):
            g, r = _split(k, w_rounds)
            idx = (pl.ds(g * _W_STREAMS, _W_STREAMS), pl.ds(r * _W_PAGES, _W_PAGES))
            pltpu.make_async_copy(buf.at[idx], o_hbm.at[idx], out_sem).start()

        def read_phase(sems):
            tail_sem, w_sem = n_groups, n_groups + 1

            def read(stream, streams, page, pages, sem):
                idx = (pl.ds(stream, streams), pl.ds(page, pages))
                return pltpu.make_async_copy(x_hbm.at[idx], buf.at[idx], sems.at[sem])

            def start_read(stream, streams, page, sem, queue):
                if queue == 1:
                    read(stream, streams - 1, page, 1, sem).start(priority=1)
                else:
                    read(stream + streams - 1, 1, page, 1, sem).start(priority=0)

            def start_round(t, queue):
                g, r = _split(t, _STREAM)
                sem = jnp.where(t >= n_rounds - _TAIL, tail_sem, g)
                start_read(_FIRST + (g - 1) * _GROUP, _GROUP, r, sem, queue)

            def wait_group(g):
                read(group_start[g], group_start[g + 1] - group_start[g], 0, _STREAM, g).wait()

            def first_round(r, _):
                start_read(0, _FIRST, r, 0, 1)
                start_read(0, _FIRST, r, 0, 0)

            def early_round(t, _):
                start_round(t, 1)
                start_round(t, 0)

            lax.fori_loop(0, _STREAM, first_round, None)
            w_copy = pltpu.make_async_copy(w_hbm, wbuf, sems.at[w_sem])
            w_copy.start()
            lax.fori_loop(_STREAM, early_rounds, early_round, None)
            w_copy.wait()

            def step(i, _):
                for g, i0 in enumerate(first_use):
                    if i0 < _READ_STEPS:
                        pl.when(i == i0)(lambda g=g: wait_group(g))
                t0 = early_rounds + i * _ROUNDS_PER_STEP
                matmul_step(i, 2 * _ROUNDS_PER_STEP,
                            lambda k: start_round(t0 + k // 2, 1 - k % 2))

            lax.fori_loop(0, _READ_STEPS, step, None)

            for g, i0 in enumerate(first_use[:-1]):
                if i0 >= _READ_STEPS:
                    wait_group(g)
            read(group_start[-2], _GROUP, 0, _STREAM - _TAIL, n_groups - 1).wait()
            lax.fori_loop(0, _W_FIRST, lambda k, _: start_write(k), None)
            read(group_start[-2], _GROUP, _STREAM - _TAIL, _TAIL, tail_sem).wait()

        pl.run_scoped(read_phase, pltpu.SemaphoreType.DMA((n_groups + 2,)))

        def step(i, _):
            k0 = _W_FIRST + (i - _READ_STEPS) * _W_PER_STEP
            matmul_step(i, _W_PER_STEP, lambda k: start_write(k0 + k))

        lax.fori_loop(_READ_STEPS, n_steps, step, None)
        lax.fori_loop(_W_FIRST + (n_steps - _READ_STEPS) * _W_PER_STEP, n_writes,
                      lambda k, _: start_write(k), None)
        pltpu.make_async_copy(buf, o_hbm, out_sem).wait()

    shape = (n_streams, _STREAM, 16, 128)
    tiles = x.reshape(2 * n_blocks, 8, 3, 128).transpose(0, 2, 1, 3)
    out = pl.pallas_call(
        kernel_function,
        in_specs=[
            pl.BlockSpec(memory_space=pl.ANY),
            pl.BlockSpec(memory_space=pl.ANY),
        ],
        out_specs=pl.BlockSpec(memory_space=pl.ANY),
        out_shape=jax.ShapeDtypeStruct(shape, x.dtype),
        scratch_shapes=[
            pltpu.VMEM(shape, x.dtype),
            pltpu.VMEM((C, C), w.dtype),
            pltpu.SemaphoreType.DMA(()),
        ],
        compiler_params=pltpu.CompilerParams(
            vmem_limit_bytes=120 * 2**20,
            disable_bounds_checks=True,
            disable_semaphore_checks=True,
        ),
    )(tiles.reshape(shape), w.reshape(C, C))
    return out.reshape(2 * n_blocks, 3, 8, 128).transpose(0, 2, 1, 3).reshape(B, H, W, C)
```

```python
import jax
import jax.numpy as jnp
from jax import lax
import jax.experimental.pallas as pl
import jax.experimental.pallas.tpu as pltpu

_STREAM = 256
_FIRST = (8, 2)
_GROUP = (11, 3)
_LAG = 26
_STEP = 128
_CHUNK = 4
_LEAD = 2
_READ_STEPS = 31
_ROUNDS_PER_STEP = 56
_TAIL = 10
_W_STREAMS = 6
_W_PAGES = 4
_W_FIRST = 22
_W_PER_STEP = 26


def _split(i, n):
    assert n & (n - 1) == 0
    return lax.shift_right_logical(i, n.bit_length() - 1), i & (n - 1)


@jax.jit
def pallas_standalone__dilated_atrous__vision_kernel(
    x: jax.Array,
    w: jax.Array,
):
    B, H, W, C = x.shape
    assert w.shape == (1, 1, C, C) and C == 384 and x.dtype.itemsize == 2
    n_blocks = B * H * W // 16
    n_streams = n_blocks * 3 // _STREAM
    n_steps = n_blocks // _STEP
    assert n_streams * _STREAM == n_blocks * 3 and n_steps * _STEP == n_blocks
    half = _STREAM // 2
    step_halves = _STEP * 3 // half
    assert step_halves * half == _STEP * 3

    first, group = sum(_FIRST), sum(_GROUP)
    n_groups = 1 + (n_streams - first) // group
    group_start = [0] + [first + g * group for g in range(n_groups)]
    assert group_start[-1] == n_streams and _TAIL % 2 == 0
    n_rounds = n_groups * _STREAM
    early_rounds = n_rounds - _READ_STEPS * _ROUNDS_PER_STEP
    assert _LAG <= _STREAM and early_rounds >= _STREAM + _LAG
    first_use = [s * _STREAM // (3 * _STEP) for s in group_start[:-1]]
    assert first_use[-1] >= _READ_STEPS
    for g, i in enumerate(first_use):
        started = early_rounds + i * _ROUNDS_PER_STEP - _LAG
        assert i >= _READ_STEPS or started >= (g + 1) * _STREAM

    w_rounds = _STREAM // _W_PAGES
    n_writes = n_streams // _W_STREAMS * w_rounds
    assert n_streams % _W_STREAMS == 0
    for i in range(_READ_STEPS, n_steps):
        last = _W_FIRST + (i - _READ_STEPS + 1) * _W_PER_STEP - 1
        assert (last // w_rounds + 1) * _W_STREAMS * _STREAM <= i * _STEP * 3

    def kernel_function(x_hbm, w_hbm, o_hbm, buf, wbuf, out_sem):
        def as_words(v):
            return pltpu.bitcast(v, jnp.int32)

        def merge(top, bottom):
            return jnp.where(lax.broadcasted_iota(jnp.int32, (8, 128), 0) < 4, top, bottom)

        def load(page, blocks):
            rows = []
            for b in blocks:
                p0, p1, p2 = (as_words(buf[page(3 * b + j)]) for j in range(3))
                cols = (merge(p0, p1), pltpu.roll(merge(p2, p0), 4, 0), merge(p1, p2))
                rows.append(jnp.concatenate([pltpu.bitcast(v, buf.dtype) for v in cols], axis=1))
            return jnp.concatenate(rows, axis=0)

        def store(page, blocks, y):
            for u, b in enumerate(blocks):
                c0, c1, c2 = (as_words(y[16 * u:16 * u + 16, 128 * j:128 * j + 128]) for j in range(3))
                c1 = pltpu.roll(c1, 4, 0)
                for j, v in enumerate((merge(c0, c1), merge(c2, c0), merge(c1, c2))):
                    buf[page(3 * b + j)] = pltpu.bitcast(v, buf.dtype)

        def matmul_step(i, n_starts, start):
            halves = [_split(i * step_halves + h, 2) for h in range(step_halves)]

            def page(n):
                stream, second = halves[n // half]
                return stream, second * half + n % half

            def blocks(chunk):
                return range(chunk * _CHUNK, (chunk + 1) * _CHUNK)

            n_chunks = _STEP // _CHUNK
            slots = iter(range(2 * n_chunks))

            def start_some():
                s = next(slots)
                lo, hi = ((t * n_starts + n_chunks) // (2 * n_chunks) for t in (s, s + 1))
                for k in range(lo, hi):
                    start(k)

            loaded = {}
            for u in range(-_LEAD, n_chunks):
                if u + _LEAD < n_chunks:
                    start_some()
                    loaded[u + _LEAD] = load(page, blocks(u + _LEAD))
                if u >= 0:
                    y = jnp.dot(loaded.pop(u), wbuf[...], preferred_element_type=jnp.float32)
                    start_some()
                    store(page, blocks(u), y.astype(buf.dtype))

        def start_write(k):
            g, r = _split(k, w_rounds)
            idx = (pl.ds(g * _W_STREAMS, _W_STREAMS), pl.ds(r * _W_PAGES, _W_PAGES))
            pltpu.make_async_copy(buf.at[idx], o_hbm.at[idx], out_sem).start()

        def read_phase(sems):
            tail_sem, w_sem = n_groups, n_groups + 1

            def read(stream, streams, page, pages, sem):
                idx = (pl.ds(stream, streams), pl.ds(page, pages))
                return pltpu.make_async_copy(x_hbm.at[idx], buf.at[idx], sems.at[sem])

            def start_read(stream, streams, r, sem, queue):
                page = r ^ (lax.shift_right_logical(r, 1) & 1)
                if queue == 1:
                    read(stream, streams[0], page, 1, sem).start(priority=1)
                else:
                    read(stream + streams[0], streams[1], page, 1, sem).start(priority=0)

            def start_first(r, queue):
                start_read(0, _FIRST, r, 0, queue)

            def start_round(t, queue):
                g, r = _split(t, _STREAM)
                sem = jnp.where(t >= n_rounds - _TAIL, tail_sem, g)
                start_read(first + (g - 1) * group, _GROUP, r, sem, queue)

            def start_rounds(lo, hi, on_1=None, on_0=None):
                def body(t, _):
                    if on_1:
                        on_1(t, 1)
                    if on_0:
                        on_0(t - _LAG, 0)
                lax.fori_loop(lo, hi, body, None)

            def wait_group(g):
                read(group_start[g], group_start[g + 1] - group_start[g], 0, _STREAM, g).wait()

            start_rounds(0, _LAG, start_first)
            start_rounds(_LAG, _STREAM, start_first, start_first)
            start_rounds(_STREAM, _STREAM + _LAG, start_round, start_first)
            w_copy = pltpu.make_async_copy(w_hbm, wbuf, sems.at[w_sem])
            w_copy.start()
            start_rounds(_STREAM + _LAG, early_rounds, start_round, start_round)
            w_copy.wait()

            def step(i, _):
                for g, i0 in enumerate(first_use):
                    if i0 < _READ_STEPS:
                        pl.when(i == i0)(lambda g=g: wait_group(g))
                t0 = early_rounds + i * _ROUNDS_PER_STEP
                matmul_step(i, 2 * _ROUNDS_PER_STEP,
                            lambda k: start_round(t0 + k // 2 - k % 2 * _LAG, 1 - k % 2))

            lax.fori_loop(0, _READ_STEPS, step, None)
            start_rounds(n_rounds, n_rounds + _LAG, on_0=start_round)

            for g, i0 in enumerate(first_use[:-1]):
                if i0 >= _READ_STEPS:
                    wait_group(g)
            read(group_start[-2], group, 0, _STREAM - _TAIL, n_groups - 1).wait()
            lax.fori_loop(0, _W_FIRST, lambda k, _: start_write(k), None)
            read(group_start[-2], group, _STREAM - _TAIL, _TAIL, tail_sem).wait()

        pl.run_scoped(read_phase, pltpu.SemaphoreType.DMA((n_groups + 2,)))

        def step(i, _):
            k0 = _W_FIRST + (i - _READ_STEPS) * _W_PER_STEP
            matmul_step(i, _W_PER_STEP, lambda k: start_write(k0 + k))

        lax.fori_loop(_READ_STEPS, n_steps, step, None)
        lax.fori_loop(_W_FIRST + (n_steps - _READ_STEPS) * _W_PER_STEP, n_writes,
                      lambda k, _: start_write(k), None)
        pltpu.make_async_copy(buf, o_hbm, out_sem).wait()

    shape = (n_streams, _STREAM, 16, 128)
    tiles = x.reshape(2 * n_blocks, 8, 3, 128).transpose(0, 2, 1, 3)
    out = pl.pallas_call(
        kernel_function,
        in_specs=[
            pl.BlockSpec(memory_space=pl.ANY),
            pl.BlockSpec(memory_space=pl.ANY),
        ],
        out_specs=pl.BlockSpec(memory_space=pl.ANY),
        out_shape=jax.ShapeDtypeStruct(shape, x.dtype),
        scratch_shapes=[
            pltpu.VMEM(shape, x.dtype),
            pltpu.VMEM((C, C), w.dtype),
            pltpu.SemaphoreType.DMA(()),
        ],
        compiler_params=pltpu.CompilerParams(
            vmem_limit_bytes=120 * 2**20,
            disable_bounds_checks=True,
            disable_semaphore_checks=True,
        ),
    )(tiles.reshape(shape), w.reshape(C, C))
    return out.reshape(2 * n_blocks, 3, 8, 128).transpose(0, 2, 1, 3).reshape(B, H, W, C)
```

```python
import jax
import jax.numpy as jnp
from jax import lax
import jax.experimental.pallas as pl
import jax.experimental.pallas.tpu as pltpu

_STREAM = 256
_FIRST = (8, 2)
_GROUP = (11, 3)
_LAG = 26
_STEP = 128
_CHUNK = 4
_LEAD = 2
_READ_STEPS = 31
_ROUNDS_PER_STEP = 56
_TAIL = 10
_W_STREAMS = 6
_W_PAGES = 4
_W_FIRST = 22
_W_PER_STEP = 26


def _split(i, n):
    assert n & (n - 1) == 0
    return lax.shift_right_logical(i, n.bit_length() - 1), i & (n - 1)


@jax.jit
def pallas_standalone__dilated_atrous__vision_kernel(
    x: jax.Array,
    w: jax.Array,
):
    B, H, W, C = x.shape
    assert w.shape == (1, 1, C, C) and C == 384 and x.dtype.itemsize == 2
    n_blocks = B * H * W // 16
    n_streams = n_blocks * 3 // _STREAM
    n_steps = n_blocks // _STEP
    assert n_streams * _STREAM == n_blocks * 3 and n_steps * _STEP == n_blocks
    half = _STREAM // 2
    step_halves = _STEP * 3 // half
    assert step_halves * half == _STEP * 3

    first, group = sum(_FIRST), sum(_GROUP)
    n_groups = 1 + (n_streams - first) // group
    group_start = [0] + [first + g * group for g in range(n_groups)]
    assert group_start[-1] == n_streams and _TAIL % 2 == 0
    n_rounds = n_groups * _STREAM
    early_rounds = n_rounds - _READ_STEPS * _ROUNDS_PER_STEP
    assert _LAG <= _STREAM and early_rounds >= _STREAM + _LAG
    first_use = [s * _STREAM // (3 * _STEP) for s in group_start[:-1]]
    assert first_use[-1] >= _READ_STEPS
    for g, i in enumerate(first_use):
        started = early_rounds + i * _ROUNDS_PER_STEP - _LAG
        assert i >= _READ_STEPS or started >= (g + 1) * _STREAM

    w_rounds = _STREAM // _W_PAGES
    n_writes = n_streams // _W_STREAMS * w_rounds
    assert n_streams % _W_STREAMS == 0
    for i in range(_READ_STEPS, n_steps):
        last = _W_FIRST + (i - _READ_STEPS + 1) * _W_PER_STEP - 1
        assert (last // w_rounds + 1) * _W_STREAMS * _STREAM <= i * _STEP * 3

    def kernel_function(x_hbm, w_hbm, o_hbm, buf, wbuf, out_sem):
        def as_words(v):
            return pltpu.bitcast(v, jnp.int32)

        def merge(top, bottom):
            return jnp.where(lax.broadcasted_iota(jnp.int32, (8, 128), 0) < 4, top, bottom)

        def load(page, blocks):
            rows = []
            for b in blocks:
                p0, p1, p2 = (as_words(buf[page(3 * b + j)]) for j in range(3))
                cols = (merge(p0, p1), pltpu.roll(merge(p2, p0), 4, 0), merge(p1, p2))
                rows.append(jnp.concatenate([pltpu.bitcast(v, buf.dtype) for v in cols], axis=1))
            return jnp.concatenate(rows, axis=0)

        def store(page, blocks, y):
            for u, b in enumerate(blocks):
                c0, c1, c2 = (as_words(y[16 * u:16 * u + 16, 128 * j:128 * j + 128]) for j in range(3))
                c1 = pltpu.roll(c1, 4, 0)
                for j, v in enumerate((merge(c0, c1), merge(c2, c0), merge(c1, c2))):
                    buf[page(3 * b + j)] = pltpu.bitcast(v, buf.dtype)

        def matmul_step(i, n_starts, start):
            halves = [_split(i * step_halves + h, 2) for h in range(step_halves)]

            def page(n):
                stream, second = halves[n // half]
                return stream, second * half + n % half

            def blocks(chunk):
                return range(chunk * _CHUNK, (chunk + 1) * _CHUNK)

            n_chunks = _STEP // _CHUNK
            slots = iter(range(2 * n_chunks))

            def start_some():
                s = next(slots)
                lo, hi = ((t * n_starts + n_chunks) // (2 * n_chunks) for t in (s, s + 1))
                for k in range(lo, hi):
                    start(k)

            loaded = {}
            for u in range(-_LEAD, n_chunks):
                if u + _LEAD < n_chunks:
                    start_some()
                    loaded[u + _LEAD] = load(page, blocks(u + _LEAD))
                if u >= 0:
                    y = jnp.dot(loaded.pop(u), wbuf[...], preferred_element_type=jnp.float32)
                    start_some()
                    store(page, blocks(u), y.astype(buf.dtype))

        def start_write(k):
            g, r = _split(k, w_rounds)
            idx = (pl.ds(g * _W_STREAMS, _W_STREAMS), pl.ds(r * _W_PAGES, _W_PAGES))
            pltpu.make_async_copy(buf.at[idx], o_hbm.at[idx], out_sem).start()

        def read_phase(sems):
            tail_sem, w_sem = n_groups, n_groups + 1

            def read(stream, streams, page, pages, sem):
                idx = (pl.ds(stream, streams), pl.ds(page, pages))
                return pltpu.make_async_copy(x_hbm.at[idx], buf.at[idx], sems.at[sem])

            def start_read(stream, streams, r, sem, queue):
                page = r ^ (lax.shift_right_logical(r, 1) & 1)
                if queue == 1:
                    read(stream, streams[0], page, 1, sem).start(priority=1)
                else:
                    read(stream + streams[0], streams[1], page, 1, sem).start(priority=0)

            def start_first(r, queue):
                start_read(0, _FIRST, r, 0, queue)

            def start_round(t, queue):
                g, r = _split(t, _STREAM)
                sem = jnp.where(t >= n_rounds - _TAIL, tail_sem, g)
                start_read(first + (g - 1) * group, _GROUP, r, sem, queue)

            def start_rounds(lo, hi, on_1=None, on_0=None):
                def body(t, _):
                    if on_1:
                        on_1(t, 1)
                    if on_0:
                        on_0(t - _LAG, 0)
                lax.fori_loop(lo, hi, body, None)

            def wait_group(g):
                read(group_start[g], group_start[g + 1] - group_start[g], 0, _STREAM, g).wait()

            start_rounds(0, _LAG, start_first)
            start_rounds(_LAG, _STREAM, start_first, start_first)
            start_rounds(_STREAM, _STREAM + _LAG, start_round, start_first)
            w_copy = pltpu.make_async_copy(w_hbm, wbuf, sems.at[w_sem])
            w_copy.start()
            start_rounds(_STREAM + _LAG, early_rounds, start_round, start_round)
            w_copy.wait()

            def step(i, _):
                for g, i0 in enumerate(first_use):
                    if i0 < _READ_STEPS:
                        pl.when(i == i0)(lambda g=g: wait_group(g))
                t0 = early_rounds + i * _ROUNDS_PER_STEP
                matmul_step(i, 2 * _ROUNDS_PER_STEP,
                            lambda k: start_round(t0 + k // 2 - k % 2 * _LAG, 1 - k % 2))

            lax.fori_loop(0, _READ_STEPS, step, None)
            start_rounds(n_rounds, n_rounds + _LAG, on_0=start_round)

            for g, i0 in enumerate(first_use[:-1]):
                if i0 >= _READ_STEPS:
                    wait_group(g)
            read(group_start[-2], group, 0, _STREAM - _TAIL, n_groups - 1).wait()
            lax.fori_loop(0, _W_FIRST, lambda k, _: start_write(k), None)
            read(group_start[-2], group, _STREAM - _TAIL, _TAIL, tail_sem).wait()

        pl.run_scoped(read_phase, pltpu.SemaphoreType.DMA((n_groups + 2,)))

        def step(i, _):
            k0 = _W_FIRST + (i - _READ_STEPS) * _W_PER_STEP
            matmul_step(i, _W_PER_STEP, lambda k: start_write(k0 + k))

        lax.fori_loop(_READ_STEPS, n_steps, step, None)
        lax.fori_loop(_W_FIRST + (n_steps - _READ_STEPS) * _W_PER_STEP, n_writes,
                      lambda k, _: start_write(k), None)
        pltpu.make_async_copy(buf, o_hbm, out_sem).wait()

    shape = (n_streams, _STREAM, 16, 128)
    tiles = x.reshape(2 * n_blocks, 8, 3, 128).transpose(0, 2, 1, 3)
    out = pl.pallas_call(
        kernel_function,
        in_specs=[
            pl.BlockSpec(memory_space=pl.ANY),
            pl.BlockSpec(memory_space=pl.ANY),
        ],
        out_specs=pl.BlockSpec(memory_space=pl.ANY),
        out_shape=jax.ShapeDtypeStruct(shape, x.dtype),
        scratch_shapes=[
            pltpu.VMEM(shape, x.dtype),
            pltpu.VMEM((C, C), w.dtype),
            pltpu.SemaphoreType.DMA(()),
        ],
        compiler_params=pltpu.CompilerParams(
            vmem_limit_bytes=120 * 2**20, disable_bounds_checks=True),
    )(tiles.reshape(shape), w.reshape(C, C))
    return out.reshape(2 * n_blocks, 3, 8, 128).transpose(0, 2, 1, 3).reshape(B, H, W, C)
```
